```python
import jax
import jax.numpy as jnp

def _softmax(x, axis=-1):
    return jax.nn.softmax(x, axis=axis)

def _gelu(x):
    return jax.nn.gelu(x, approximate=True)

def _silu(x):
    return jax.nn.silu(x)

def _sigmoid(x):
    return jax.nn.sigmoid(x)

def _layernorm(x, axis=-1, eps=1e-05):
    m = jnp.mean(x, axis=axis, keepdims=True)
    v = jnp.var(x, axis=axis, keepdims=True)
    return (x - m) / jnp.sqrt(v + eps)

def _scatter_add(tgt, idx, src, axis=0):
    return tgt.at[idx].add(src)

def _segment_sum(src, seg, n):
    return jax.ops.segment_sum(src, seg, n)

class _Rng:

    def __init__(self, key):
        self._k = key

    def _next(self):
        self._k, sub = jax.random.split(self._k)
        return sub

    def normal(self, shape):
        return jax.random.normal(self._next(), shape, dtype=jnp.bfloat16)

    def randint(self, lo, hi, shape):
        return jax.random.randint(self._next(), shape, lo, hi, dtype=jnp.int32)

    def uniform(self, shape, lo=0.0, hi=1.0):
        return jax.random.uniform(self._next(), shape, jnp.bfloat16, lo, hi)

    def permutation(self, n):
        return jax.random.permutation(self._next(), n)
kernel_name = 'adaLN_cond__sliding_block_cached__dense_activation_mish__decode'

def setup_inputs():
    _rng = _Rng(jax.random.key(int.from_bytes(__import__("os").urandom(4), "little")))
    _w = lambda a: (lambda t: t.astype(jnp.bfloat16) if jnp.issubdtype(t.dtype, jnp.floating) else t)(jnp.asarray(a))

    def _A_setup():
        B, Sq, D = (1, 1, 640)
        Hq, Hkv, Sk, Dh = (32, 32, 32768, 192)
        assert Hq % Hkv == 0, (Hq, Hkv)
        return {'x': _w((lambda *s: _rng.normal(s) * 0.05)(B, Sq, D)), 'k_cache': _w((lambda *s: _rng.normal(s) * 0.05)(B, Hkv, Sk, Dh)), 'v_cache': _w((lambda *s: _rng.normal(s) * 0.05)(B, Hkv, Sk, Dh)), 'wq': _w((lambda *s: _rng.normal(s) * 0.05)(D, Hq * Dh) * D ** (-0.5)), 'wo': _w((lambda *s: _rng.normal(s) * 0.05)(Hq * Dh, D) * (Hq * Dh) ** (-0.5))}
    _A_in = _A_setup()

    def _B_setup():
        B, S, D, F = (1, 1, 640, 1536)
        return {'x': _w((lambda *s: _rng.normal(s) * 0.05)(B, S, D)), 'w1': _w((lambda *s: _rng.normal(s) * 0.05)(D, F) * D ** (-0.5)), 'b1': _w((lambda *s: _rng.normal(s) * 0.05)(F)), 'w2': _w((lambda *s: _rng.normal(s) * 0.05)(F, D) * F ** (-0.5))}
    _B_in = _B_setup()
    return {'A_x': _A_in['x'], 'A_k_cache': _A_in['k_cache'], 'A_v_cache': _A_in['v_cache'], 'A_wq': _A_in['wq'], 'A_wo': _A_in['wo'], 'B_x': _B_in['x'], 'B_w1': _B_in['w1'], 'B_b1': _B_in['b1'], 'B_w2': _B_in['w2'], 'c': _w((lambda *s: _rng.normal(s) * 0.05)(1, 640)), 'w_mod': _w((lambda *s: _rng.normal(s) * 0.05)(640, 6 * 640) * 640 ** (-0.5))}

def reference(A_x, A_k_cache, A_v_cache, A_wq, A_wo, B_x, B_w1, B_b1, B_w2, c, w_mod):

    def _A_ref(x, k_cache, v_cache, wq, wo):
        B, Sq, D = x.shape
        Hq, Dh = (32, 192)
        Hkv, Sk = (k_cache.shape[1], k_cache.shape[2])
        W = min(4096, max(256, Sk // 4))
        rep = Hq // Hkv
        q = (lambda x, *d: x.transpose(*d))((x @ wq).reshape(B, Sq, Hq, Dh), 0, 2, 1, 3)
        k = jnp.repeat(k_cache[:, :, Sk - W:, :], rep, axis=1)
        v = jnp.repeat(v_cache[:, :, Sk - W:, :], rep, axis=1)
        scores = jnp.einsum('bhqd,bhkd->bhqk', q, k) * Dh ** (-0.5)
        p = _softmax(scores, axis=-1)
        o = jnp.einsum('bhqk,bhkd->bhqd', p, v)
        return (lambda x, *d: x.transpose(*d))(o, 0, 2, 1, 3).reshape(B, Sq, Hq * Dh) @ wo

    def _B_ref(x, w1, b1, w2):
        h = jnp.einsum('bsd,df->bsf', x, w1) + b1
        sp = jnp.log1p(jnp.exp(-jnp.abs(h))) + jnp.where(h > 0, h, jnp.zeros_like(h))
        act = h * jnp.tanh(sp)
        return jnp.einsum('bsf,fd->bsd', act, w2)
    x = A_x
    mod = (_silu(c) @ w_mod).reshape(c.shape[0], 6, 1, -1)
    sa, ca, ga, sb, cb, gb = (mod[:, 0].copy(), mod[:, 1].copy(), mod[:, 2].copy(), mod[:, 3].copy(), mod[:, 4].copy(), mod[:, 5].copy())
    h = _layernorm(x, axis=-1) * (1 + ca) + sa
    x = x + ga * _A_ref(h, A_k_cache, A_v_cache, A_wq, A_wo)
    h = _layernorm(x, axis=-1) * (1 + cb) + sb
    x = x + gb * _B_ref(h, B_w1, B_b1, B_w2)
    return x
```

```python
import functools

import jax
import jax.numpy as jnp
from jax.experimental import pallas as pl
from jax.experimental.pallas import tpu as pltpu

F32 = jnp.float32
BF16 = jnp.bfloat16

HQ, DH = 32, 192
G = 8
GR = G * DH
NG = HQ // G
EPS = 1e-5


def _layernorm(x):
    m = jnp.mean(x, axis=-1, keepdims=True)
    d = x - m
    v = jnp.mean(d * d, axis=-1, keepdims=True)
    return d / jnp.sqrt(v + EPS)


def _dot(a, b):
    return jnp.dot(a, b, preferred_element_type=F32)


def _dot_nt(a, b):
    return jax.lax.dot_general(a, b, (((1,), (1,)), ((), ())), preferred_element_type=F32)


def _make(name="adaln_attn_mish", C=512, n_wo=4, n_w2=4, bg_prio=1):
    def kernel(x_hbm, kt_hbm, vt_hbm, wq_hbm, wo_hbm, w1_hbm, b1_hbm, w2_hbm, c_hbm, wm_hbm,
               o_ref,
               x_v, c_v, b1_v, wma_v, wmb_v, wq_v, wo_v, w1_v, w2_v, ring, q_v, s_v, p_v, a_v,
               ring_sem, w_sem, wo_sem, w2_sem):
        D = x_v.shape[-1]
        SK = kt_hbm.shape[1]
        W = s_v.shape[0] * s_v.shape[2]
        NC = W // C
        FF = w1_v.shape[1]
        wo_rows = wo_v.shape[0] // n_wo
        w2_rows = FF // n_w2

        def kv_copy(src, g, c):
            return pltpu.make_async_copy(
                src.at[pl.ds(pl.multiple_of(g * GR, GR), GR), pl.ds(pl.multiple_of(SK - W + c * C, C), C)],
                ring.at[c], ring_sem.at[c])

        cp_c = pltpu.make_async_copy(c_hbm, c_v, w_sem.at[0])
        cp_x = pltpu.make_async_copy(x_hbm, x_v, w_sem.at[1])
        cp_wma = pltpu.make_async_copy(wm_hbm.at[:, pl.ds(0, 2 * D)], wma_v, w_sem.at[2])
        cp_wq = pltpu.make_async_copy(wq_hbm, wq_v, w_sem.at[3])
        cp_b1 = pltpu.make_async_copy(b1_hbm, b1_v, w_sem.at[4])
        cp_wmb = pltpu.make_async_copy(wm_hbm.at[:, pl.ds(2 * D, 4 * D)], wmb_v, w_sem.at[5])
        cp_w1 = pltpu.make_async_copy(w1_hbm, w1_v, w_sem.at[6])
        cp_wo = [pltpu.make_async_copy(wo_hbm.at[pl.ds(i * wo_rows, wo_rows)], wo_v.at[pl.ds(i * wo_rows, wo_rows)],
                                       wo_sem.at[i]) for i in range(n_wo)]
        cp_w2 = [pltpu.make_async_copy(w2_hbm.at[pl.ds(i * w2_rows, w2_rows)], w2_v.at[pl.ds(i * w2_rows, w2_rows)],
                                       w2_sem.at[i]) for i in range(n_w2)]

        cp_wma.start()
        cp_c.start()
        cp_x.start()
        cp_b1.start()
        cp_wq.start()
        cp_wmb.start()
        for c in range(NC):
            kv_copy(kt_hbm, 0, c).start()
        if bg_prio:
            for cp in cp_wo:
                cp.start(priority=1)
            cp_w1.start(priority=1)
            for cp in cp_w2:
                cp.start(priority=1)

        cp_c.wait()
        cp_x.wait()
        cv = c_v[...].astype(F32)
        sc = (cv * jax.nn.sigmoid(cv)).astype(BF16)
        x = x_v[0].astype(F32)
        xn = _layernorm(x)
        cp_wma.wait()
        moda = _dot(sc, wma_v[...])
        h = (xn * (1.0 + moda[:, D:]) + moda[:, :D]).astype(BF16)
        cp_wq.wait()
        row = jax.lax.broadcasted_iota(jnp.int32, (G, GR), 0)
        col = jax.lax.broadcasted_iota(jnp.int32, (G, GR), 1)
        own = (col >= row * DH) & (col < (row + 1) * DH)
        for g in range(NG):
            q = _dot(h, wq_v[:, g * GR:(g + 1) * GR])
            q_v[g] = jnp.where(own, jnp.broadcast_to(q, (G, GR)), 0.0)
        cp_wmb.wait()
        modb = _dot(sc, wmb_v[...])
        cp_b1.wait()

        scale = DH ** -0.5

        def group(g, carry):
            qg = q_v[g].astype(BF16)

            def k_step(c, carry):
                kv_copy(kt_hbm, g, c).wait()
                s_v[c] = _dot(qg, ring[c]) * scale
                kv_copy(vt_hbm, g, c).start()
                return carry

            jax.lax.fori_loop(0, NC, k_step, 0)

            s = s_v[...]
            m = jnp.max(jnp.max(s, axis=0), axis=-1, keepdims=True)
            e = jnp.exp(s - m[None])
            l = jnp.sum(jnp.sum(e, axis=0), axis=-1, keepdims=True)
            p_v[...] = e

            def v_step(c, acc):
                kv_copy(vt_hbm, g, c).wait()
                acc = acc + _dot_nt(p_v[c].astype(BF16), ring[c])

                @pl.when(g + 1 < NG)
                def _():
                    kv_copy(kt_hbm, g + 1, c).start()

                if not bg_prio:
                    @pl.when((g + 1 == NG) & (c == 0))
                    def _():
                        for cp in cp_wo:
                            cp.start()
                        cp_w1.start()
                        for cp in cp_w2:
                            cp.start()
                return acc

            acc = jax.lax.fori_loop(0, NC, v_step, jnp.zeros((G, GR), F32))
            a_v[g] = jnp.sum(jnp.where(own, acc / l, 0.0), axis=0, keepdims=True)
            return carry

        jax.lax.fori_loop(0, NG, group, 0)

        a = jnp.concatenate([a_v[g] for g in range(NG)], axis=1).astype(BF16)
        y = jnp.zeros((1, D), F32)
        for i in range(n_wo):
            cp_wo[i].wait()
            y = y + _dot(a[:, i * wo_rows:(i + 1) * wo_rows], wo_v[i * wo_rows:(i + 1) * wo_rows, :])
        ga, sb, cb, gb = (modb[:, i * D:(i + 1) * D] for i in range(4))
        x1 = x + ga * y
        h2 = (_layernorm(x1) * (1.0 + cb) + sb).astype(BF16)
        b1 = b1_v[...].astype(F32)
        b1 = jnp.concatenate([b1[j:j + 1, :] for j in range(FF // 128)], axis=1)
        cp_w1.wait()
        u = _dot(h2, w1_v[...]) + b1
        sp = jnp.log1p(jnp.exp(-jnp.abs(u))) + jnp.where(u > 0, u, 0.0)
        act = (u * jnp.tanh(sp)).astype(BF16)
        z = jnp.zeros((1, D), F32)
        for i in range(n_w2):
            cp_w2[i].wait()
            z = z + _dot(act[:, i * w2_rows:(i + 1) * w2_rows], w2_v[i * w2_rows:(i + 1) * w2_rows, :])
        o_ref[0] = (x1 + gb * z).astype(o_ref.dtype)

    def fn(A_x, A_k_cache, A_v_cache, A_wq, A_wo, B_x, B_w1, B_b1, B_w2, c, w_mod):
        del B_x
        _, hkv, sk, dh = A_k_cache.shape
        D = A_x.shape[-1]
        FF = B_w1.shape[1]
        W = min(4096, max(256, sk // 4))
        NC = W // C
        kt = jnp.swapaxes(A_k_cache, 2, 3).reshape(hkv * dh, sk)
        vt = jnp.swapaxes(A_v_cache, 2, 3).reshape(hkv * dh, sk)
        b1 = B_b1.reshape(FF // 128, 128)
        hbm = pl.BlockSpec(memory_space=pltpu.HBM)
        return pl.pallas_call(
            kernel, name=name,
            out_shape=jax.ShapeDtypeStruct(A_x.shape, A_x.dtype),
            in_specs=[hbm] * 10,
            out_specs=pl.BlockSpec(memory_space=pltpu.VMEM),
            scratch_shapes=[
                pltpu.VMEM(A_x.shape, BF16), pltpu.VMEM(c.shape, BF16), pltpu.VMEM(b1.shape, BF16),
                pltpu.VMEM((D, 2 * D), BF16), pltpu.VMEM((D, 4 * D), BF16),
                pltpu.VMEM(A_wq.shape, BF16), pltpu.VMEM(A_wo.shape, BF16),
                pltpu.VMEM(B_w1.shape, BF16), pltpu.VMEM(B_w2.shape, BF16),
                pltpu.VMEM((NC, GR, C), BF16),
                pltpu.VMEM((NG, G, GR), F32), pltpu.VMEM((NC, G, C), F32), pltpu.VMEM((NC, G, C), F32),
                pltpu.VMEM((NG, 1, GR), F32),
                pltpu.SemaphoreType.DMA((NC,)), pltpu.SemaphoreType.DMA((7,)),
                pltpu.SemaphoreType.DMA((n_wo,)), pltpu.SemaphoreType.DMA((n_w2,)),
            ],
            compiler_params=pltpu.CompilerParams(vmem_limit_bytes=64 * 1024 * 1024),
        )(A_x, kt, vt, A_wq, A_wo, B_w1, b1, B_w2, c, w_mod)

    return fn


@jax.jit
def pallas_adaLN_cond__sliding_block_cached__dense_activation_mish__decode_kernel(
    A_x, A_k_cache, A_v_cache, A_wq, A_wo, B_x, B_w1, B_b1, B_w2, c, w_mod):
    return _make()(A_x, A_k_cache, A_v_cache, A_wq, A_wo, B_x, B_w1, B_b1, B_w2, c, w_mod)
```

```python
import contextlib

import jax
import jax.numpy as jnp
from jax.experimental import pallas as pl
from jax.experimental.pallas import tpu as pltpu

F32 = jnp.float32
BF16 = jnp.bfloat16

HQ, DH = 32, 192
G = 8
GR = G * DH
NG = HQ // G
NC = 4
EPS = 1e-5


def _layernorm(x):
    m = jnp.mean(x, axis=-1, keepdims=True)
    d = x - m
    v = jnp.mean(d * d, axis=-1, keepdims=True)
    return d / jnp.sqrt(v + EPS)


def _dot(a, b):
    return jnp.dot(a, b, preferred_element_type=F32)


def _dot_nt(a, b):
    return jax.lax.dot_general(a, b, (((1,), (1,)), ((), ())), preferred_element_type=F32)


def _loop(n, body):
    def step(i, carry):
        body(i)
        return carry
    jax.lax.fori_loop(0, n, step, 0)


def _deal(n, piece):
    def pair(i):
        piece(2 * i).start(priority=0)
        piece(2 * i + 1).start(priority=1)
    _loop(n // 2, pair)
    if n % 2:
        piece(n - 1).start(priority=0)


def _spread(i, n, ways):
    assert n % ways == 0
    return (i % ways) * (n // ways) + i // ways


def _make(name="adaln_attn_mish", w2_split=(1024, 384, 128), nosem=0, scopes=0, kv_rows=32,
         wq_p=(8, 2048, 5), wm_p=(8, 1920, 5), wo_p=(16, 640, 8), w1_p=(8, 1536, 4), w2_p=(16, 640, 4),
         wo_a=3072, nobc=0, skipkv=0, kv_unroll=1):

    def scope(n):
        return jax.named_scope(n) if scopes else contextlib.nullcontext()

    def kernel(x_hbm, kt_hbm, vt_hbm, wq_hbm, wo_hbm, w1_hbm, b1_hbm, w2_hbm, c_hbm, wm_hbm,
               o_ref,
               x_v, c_v, b1_v, wm_v, wq_v, woa_v, wob_v, w1_v, ring, q_v, s_v, p_v, a_v, y_v, sem, *w2_v):
        D = x_v.shape[-1]
        SK = kt_hbm.shape[1]
        C = ring.shape[3]
        W = 2 * NC * C
        FF = w1_v.shape[1]
        HO = woa_v.shape[0]
        w2_off = [sum(w2_split[:i]) for i in range(len(w2_split))]

        def fetch(src, row0, dst, s, pat):
            r, c, ways = pat
            nr, nc = dst.shape[0] // r, dst.shape[1] // c
            assert nr * r == dst.shape[0] and nc * c == dst.shape[1], (dst.shape, pat)
            while nr % ways:
                ways -= 1
            n = nr // ways
            k = [0]

            def sweep(i, cc):
                for w in range(ways):
                    rr = i * r + w * n * r
                    if not isinstance(rr, int):
                        rr = pl.multiple_of(rr, r)
                    pltpu.make_async_copy(src.at[pl.ds(row0 + rr, r), pl.ds(cc, c)],
                                          dst.at[pl.ds(rr, r), pl.ds(cc, c)], sem.at[s]).start(priority=k[0] % 2)
                    k[0] += 1

            if ways % 2 == 0:
                for j in range(nc):
                    _loop(n, lambda i: sweep(i, j * c))
            else:
                assert n % 2 == 0
                for j in range(nc):
                    _loop(n // 2, lambda i: (sweep(2 * i, j * c), sweep(2 * i + 1, j * c)))

        def landed(dst, s):
            pltpu.make_async_copy(dst, dst, sem.at[s]).wait()

        def fetch_kv(src, g, c):
            slot = c % 2
            srcs = [src.at[pl.ds(pl.multiple_of(g * GR, GR), GR),
                           pl.ds(pl.multiple_of(SK - W + half * (W // 2) + c * C, C), C)] for half in range(2)]
            dsts = [ring.at[slot, half] for half in range(2)]

            def step(i):
                for u in range(kv_unroll):
                    r = pl.multiple_of((i * kv_unroll + u) * kv_rows, kv_rows)
                    for half in range(2):
                        pltpu.make_async_copy(srcs[half].at[pl.ds(r, kv_rows)], dsts[half].at[pl.ds(r, kv_rows)],
                                              sem.at[slot]).start(priority=half)
            _loop(GR // kv_rows // kv_unroll, step)

        small = [pltpu.make_async_copy(c_hbm, c_v, sem.at[2]),
                 pltpu.make_async_copy(x_hbm, x_v, sem.at[2]),
                 pltpu.make_async_copy(b1_hbm, b1_v, sem.at[2])]
        fetch(wm_hbm, 0, wm_v, 2, wm_p)
        for cp in small:
            cp.start()
        fetch(wq_hbm, 0, wq_v, 3, wq_p)

        with scope("s0_head_wait"):
            for cp in small:
                cp.wait()
            landed(wm_v, 2)
        cv = c_v[...].astype(F32)
        sc = (cv * jax.nn.sigmoid(cv)).astype(BF16)
        x = x_v[0].astype(F32)
        mod = _dot(sc, wm_v[...])
        sa, ca, ga, sb, cb, gb = (mod[:, i * D:(i + 1) * D] for i in range(6))
        h = (_layernorm(x) * (1.0 + ca) + sa).astype(BF16)
        fetch_kv(kt_hbm, 0, 0)
        with scope("s1_wq_wait"):
            landed(wq_v, 3)
        row = jax.lax.broadcasted_iota(jnp.int32, (G, GR), 0)
        col = jax.lax.broadcasted_iota(jnp.int32, (G, GR), 1)
        own = (col >= row * DH) & (col < (row + 1) * DH)
        for g in range(NG):
            q = _dot(h, wq_v[:, g * GR:(g + 1) * GR])
            q_v[g] = jnp.where(own, jnp.broadcast_to(q, (G, GR)), 0.0)

        scale = DH ** -0.5

        def group(g):
            qg = q_v[g].astype(BF16)

            def k_step(c):
                @pl.when(c + 1 < NC)
                def _():
                    fetch_kv(kt_hbm, g, c + 1)

                @pl.when(c + 1 == NC)
                def _():
                    fetch_kv(vt_hbm, g, 0)

                landed(ring.at[c % 2], c % 2)
                for half in range(2):
                    if skipkv: s_v[c, half] = jnp.zeros((G, C), F32)
                    else: s_v[c, half] = _dot(qg, ring[c % 2, half]) * scale

            _loop(NC, k_step)

            s = s_v[...]
            m = jnp.max(jnp.max(s, axis=(0, 1)), axis=-1, keepdims=True)
            e = jnp.exp(s - m[None, None])
            l = jnp.sum(jnp.sum(e, axis=(0, 1)), axis=-1, keepdims=True)
            p_v[...] = e

            def v_step(c, acc):
                @pl.when(c + 1 < NC)
                def _():
                    fetch_kv(vt_hbm, g, c + 1)

                @pl.when((c + 1 == NC) & (g + 1 < NG))
                def _():
                    fetch_kv(kt_hbm, g + 1, 0)

                @pl.when((c + 1 == NC) & (g + 1 == NG))
                def _():
                    fetch(wo_hbm, 0, woa_v, 2, wo_p)

                landed(ring.at[c % 2], c % 2)
                for half in range(2):
                    if not skipkv: acc = acc + _dot_nt(p_v[c, half].astype(BF16), ring[c % 2, half])
                return acc

            acc = jax.lax.fori_loop(0, NC, v_step, jnp.zeros((G, GR), F32))
            a_v[g] = jnp.sum(jnp.where(own, acc / l, 0.0), axis=0, keepdims=True)

        with scope("s2_attn"):
            _loop(NG, group)

        fetch(wo_hbm, HO, wob_v, 3, wo_p)
        fetch(w1_hbm, 0, w1_v, 3, w1_p)
        a = jnp.concatenate([a_v[g] for g in range(NG)], axis=1).astype(BF16)
        with scope("s4_woa_wait"):
            landed(woa_v, 2)
        y_v[...] = _dot(a[:, :HO], woa_v[...])
        assert len(w2_split) <= 3
        for i in range(len(w2_split)):
            fetch(w2_hbm, w2_off[i], w2_v[i], i, w2_p)
        with scope("s5_wob_wait"):
            landed(wob_v, 3)
            landed(w1_v, 3)
        y = y_v[...] + _dot(a[:, HO:], wob_v[...])
        x1 = x + ga * y
        h2 = (_layernorm(x1) * (1.0 + cb) + sb).astype(BF16)
        b1 = b1_v[...].astype(F32)
        b1 = jnp.concatenate([b1[j:j + 1, :] for j in range(FF // 128)], axis=1)
        u = _dot(h2, w1_v[...]) + b1
        sp = jnp.log1p(jnp.exp(-jnp.abs(u))) + jnp.where(u > 0, u, 0.0)
        act = (u * jnp.tanh(sp)).astype(BF16)
        y_v[...] = x1
        for i in range(len(w2_split)):
            with scope(f"s7_w2_{i}_wait"):
                landed(w2_v[i], i)
            out = y_v[...] + gb * _dot(act[:, w2_off[i]:w2_off[i] + w2_split[i]], w2_v[i][...])
            if i + 1 < len(w2_split):
                y_v[...] = out
        with scope("s8_out"):
            o_ref[0] = out.astype(o_ref.dtype)

    def fn(A_x, A_k_cache, A_v_cache, A_wq, A_wo, B_x, B_w1, B_b1, B_w2, c, w_mod):
        del B_x
        _, hkv, sk, dh = A_k_cache.shape
        D = A_x.shape[-1]
        FF = B_w1.shape[1]
        W = min(4096, max(256, sk // 4))
        C = W // (2 * NC)
        kt = jnp.swapaxes(A_k_cache, 2, 3).reshape(hkv * dh, sk)
        vt = jnp.swapaxes(A_v_cache, 2, 3).reshape(hkv * dh, sk)
        b1 = B_b1.reshape(FF // 128, 128)
        hbm = pl.BlockSpec(memory_space=pltpu.HBM)
        return pl.pallas_call(
            kernel, name=name,
            out_shape=jax.ShapeDtypeStruct(A_x.shape, A_x.dtype),
            in_specs=[hbm] * 10,
            out_specs=pl.BlockSpec(memory_space=pltpu.VMEM),
            scratch_shapes=[
                pltpu.VMEM(A_x.shape, BF16), pltpu.VMEM(c.shape, BF16), pltpu.VMEM(b1.shape, BF16),
                pltpu.VMEM(w_mod.shape, BF16),
                pltpu.VMEM(A_wq.shape, BF16), pltpu.VMEM((wo_a, D), BF16),
                pltpu.VMEM((A_wo.shape[0] - wo_a, D), BF16),
                pltpu.VMEM(B_w1.shape, BF16),
                pltpu.VMEM((2, 2, GR, C), BF16),
                pltpu.VMEM((NG, G, GR), F32), pltpu.VMEM((NC, 2, G, C), F32), pltpu.VMEM((NC, 2, G, C), F32),
                pltpu.VMEM((NG, 1, GR), F32), pltpu.VMEM((1, D), F32),
                pltpu.SemaphoreType.DMA((4,)),
            ] + [pltpu.VMEM((r, D), BF16) for r in w2_split],
            compiler_params=pltpu.CompilerParams(vmem_limit_bytes=64 * 1024 * 1024,
                                                 disable_semaphore_checks=bool(nosem), disable_bounds_checks=bool(nobc)),
        )(A_x, kt, vt, A_wq, A_wo, B_w1, b1, B_w2, c, w_mod)

    return fn


@jax.jit
def pallas_adaLN_cond__sliding_block_cached__dense_activation_mish__decode_kernel(
    A_x, A_k_cache, A_v_cache, A_wq, A_wo, B_x, B_w1, B_b1, B_w2, c, w_mod):
    return _make()(A_x, A_k_cache, A_v_cache, A_wq, A_wo, B_x, B_w1, B_b1, B_w2, c, w_mod)
```

```python
import contextlib
import functools

import jax
import jax.numpy as jnp
from jax.experimental import pallas as pl
from jax.experimental.pallas import tpu as pltpu

F32 = jnp.float32
BF16 = jnp.bfloat16

HQ, DH = 32, 192
G = 8
GR = G * DH
NG = HQ // G
NC = 4
KV_ROWS = 32
EPS = 1e-5

S_SMALL, S_WM, S_WQ, S_WOA, S_WOB, S_W1, S_W2 = range(2, 9)


def _layernorm(x):
    m = jnp.mean(x, axis=-1, keepdims=True)
    d = x - m
    v = jnp.mean(d * d, axis=-1, keepdims=True)
    return d / jnp.sqrt(v + EPS)


def _dot(a, b):
    return jnp.dot(a, b, preferred_element_type=F32)


def _dot_nt(a, b):
    return jax.lax.dot_general(a, b, (((1,), (1,)), ((), ())), preferred_element_type=F32)


def _loop(n, body):
    def step(i, carry):
        body(i)
        return carry
    jax.lax.fori_loop(0, n, step, 0)


def _make(name="adaln_attn_mish", w2_split=(1024, 384, 128), wo_a=4608, vpu_tail=0, scopes=0, w2_rows=16, w2_a=768):

    def scope(n):
        return jax.named_scope(n) if scopes else contextlib.nullcontext()

    def body(x_hbm, kt_hbm, vt_hbm, wq_hbm, wo_hbm, w1_hbm, b1_hbm, w2_hbm, c_hbm, wm_hbm,
             o_ref,
             x_v, c_v, b1_v, wm_v, wq_v, woa_v, wob_v, w1_v, kv_v, q_v, s_v, p_v, a_v, y_v, *w2_v, sem):
        D = x_v.shape[-1]
        FF = w1_v.shape[1]
        SK = kt_hbm.shape[1]
        C = kv_v.shape[3]
        W = 2 * NC * C

        def fetch(src, row0, dst, s, rows, cols, ways):
            n = dst.shape[0] // (rows * ways)
            nc = dst.shape[1] // cols
            assert (n * rows * ways, nc * cols) == dst.shape and (ways * nc) % 2 == 0

            def sweep(i):
                for j in range(nc):
                    for w in range(ways):
                        r = pl.multiple_of((w * n + i) * rows, rows)
                        pltpu.make_async_copy(src.at[pl.ds(row0 + r, rows), pl.ds(j * cols, cols)],
                                              dst.at[pl.ds(r, rows), pl.ds(j * cols, cols)],
                                              sem.at[s]).start(priority=(j * ways + w) % 2)
            _loop(n, sweep)

        def fetch_kv(src, g, c):
            rows = pl.ds(pl.multiple_of(g * GR, GR), GR)
            strips = [src.at[rows, pl.ds(pl.multiple_of(SK - W + half * (W // 2) + c * C, C), C)]
                      for half in range(2)]

            def step(i):
                r = pl.ds(pl.multiple_of(i * KV_ROWS, KV_ROWS), KV_ROWS)
                for half in range(2):
                    pltpu.make_async_copy(strips[half].at[r], kv_v.at[c % 2, half, r],
                                          sem.at[c % 2]).start(priority=half)
            _loop(GR // KV_ROWS, step)

        def landed(dst, s):
            pltpu.make_async_copy(dst, dst, sem.at[s]).wait()

        small = [pltpu.make_async_copy(src, dst, sem.at[S_SMALL])
                 for src, dst in ((c_hbm, c_v), (x_hbm, x_v), (b1_hbm, b1_v))]
        fetch(wm_hbm, 0, wm_v, S_WM, 8, 1280, 10)
        for cp in small:
            cp.start()
        fetch(wq_hbm, 0, wq_v, S_WQ, 8, 2048, 20)

        for cp in small:
            cp.wait()
        landed(wm_v, S_WM)
        cv = c_v[...].astype(F32)
        mod = _dot((cv * jax.nn.sigmoid(cv)).astype(BF16), wm_v[...])
        sa, ca, ga, sb, cb, gb = (mod[:, i * D:(i + 1) * D] for i in range(6))
        x = x_v[0].astype(F32)
        h = (_layernorm(x) * (1.0 + ca) + sa).astype(BF16)

        fetch_kv(kt_hbm, 0, 0)
        landed(wq_v, S_WQ)
        row = jax.lax.broadcasted_iota(jnp.int32, (G, GR), 0)
        col = jax.lax.broadcasted_iota(jnp.int32, (G, GR), 1)
        own = (col >= row * DH) & (col < (row + 1) * DH)
        for g in range(NG):
            q = _dot(h, wq_v[:, g * GR:(g + 1) * GR])
            q_v[g] = jnp.where(own, jnp.broadcast_to(q, (G, GR)), 0.0)

        def group(g):
            qg = q_v[g].astype(BF16)

            def k_step(c):
                @pl.when(c + 1 < NC)
                def _():
                    fetch_kv(kt_hbm, g, c + 1)

                @pl.when(c + 1 == NC)
                def _():
                    fetch_kv(vt_hbm, g, 0)

                landed(kv_v.at[c % 2], c % 2)
                for half in range(2):
                    s_v[c, half] = _dot(qg, kv_v[c % 2, half]) * DH ** -0.5

            _loop(NC, k_step)

            s = s_v[...]
            m = jnp.max(jnp.max(s, axis=(0, 1)), axis=-1, keepdims=True)
            e = jnp.exp(s - m[None, None])
            l = jnp.sum(jnp.sum(e, axis=(0, 1)), axis=-1, keepdims=True)
            p_v[...] = e

            def v_step(c, acc):
                @pl.when(c + 1 < NC)
                def _():
                    fetch_kv(vt_hbm, g, c + 1)

                @pl.when((c + 1 == NC) & (g + 1 < NG))
                def _():
                    fetch_kv(kt_hbm, g + 1, 0)

                @pl.when((c + 1 == NC) & (g + 1 == NG))
                def _():
                    fetch(wo_hbm, 0, woa_v, S_WOA, 16, D, 8)

                landed(kv_v.at[c % 2], c % 2)
                for half in range(2):
                    acc = acc + _dot_nt(p_v[c, half].astype(BF16), kv_v[c % 2, half])
                return acc

            acc = jax.lax.fori_loop(0, NC, v_step, jnp.zeros((G, GR), F32))
            a_v[g] = jnp.sum(jnp.where(own, acc / l, 0.0), axis=0, keepdims=True)

        _loop(NG, group)

        HA = woa_v.shape[0]
        fetch(wo_hbm, HA, wob_v, S_WOB, 16, D, 8)
        fetch(w1_hbm, 0, w1_v, S_W1, 8, FF, 4)
        a = jnp.concatenate([a_v[g] for g in range(NG)], axis=1).astype(BF16)
        landed(woa_v, S_WOA)
        y_v[...] = _dot(a[:, :HA], woa_v[...])

        edges = [sum(v.shape[0] for v in w2_v[:i]) for i in range(len(w2_v) + 1)]

        def w2_copy(r):
            i = max(j for j in range(len(w2_v)) if edges[j] <= r)
            return pltpu.make_async_copy(w2_hbm.at[pl.ds(r, w2_rows)], w2_v[i].at[pl.ds(r - edges[i], w2_rows)],
                                         sem.at[S_W2 + i])
        for r in range(0, max(w2_a, FF - w2_a), w2_rows):
            if r < w2_a:
                w2_copy(r).start(priority=0)
            if w2_a + r < FF:
                w2_copy(w2_a + r).start(priority=1)

        with scope("s5_wob_wait"):
            landed(wob_v, S_WOB)
        x1 = x + ga * (y_v[...] + _dot(a[:, HA:], wob_v[...]))
        h2 = (_layernorm(x1) * (1.0 + cb) + sb).astype(BF16)
        y_v[...] = x1
        b1 = b1_v[...].astype(F32)
        b1 = jnp.concatenate([b1[j:j + 1, :] for j in range(FF // 128)], axis=1)
        with scope("s6_w1_wait"):
            landed(w1_v, S_W1)
        u = _dot(h2, w1_v[...]) + b1
        sp = jnp.log1p(jnp.exp(-jnp.abs(u))) + jnp.where(u > 0, u, 0.0)
        act = (u * jnp.tanh(sp)).astype(BF16)
        if vpu_tail:
            n_last = w2_v[-1].shape[0]
            coef = jnp.broadcast_to(act[:, FF - 128:].astype(F32), (128, 128)).T[128 - n_last:]
            p_v[0, 0, :, :] = jnp.concatenate([coef[8 * i:8 * i + 8] for i in range(4)], axis=1)
            p_v[0, 1, :, :] = jnp.concatenate([coef[8 * i:8 * i + 8] for i in range(4, 8)], axis=1)
            p_v[1, 0, :, :] = jnp.concatenate([coef[8 * i:8 * i + 8] for i in range(8, 12)], axis=1)
            p_v[1, 1, :, :] = jnp.concatenate([coef[8 * i:8 * i + 8] for i in range(12, 16)], axis=1)
        for i in range(len(w2_v)):
            with scope(f"s7_w2_{i}_wait"):
                landed(w2_v[i], S_W2 + i)
            if vpu_tail and i + 1 == len(w2_v):
                coef = jnp.concatenate([p_v[k // 8, (k // 4) % 2, :, (k % 4) * 128:(k % 4 + 1) * 128] for k in range(16)], axis=0)
                z = jnp.concatenate(
                    [jnp.sum(w2_v[i][:, j * 128:(j + 1) * 128].astype(F32) * coef, axis=0, keepdims=True)
                     for j in range(D // 128)], axis=1)
            else:
                z = _dot(act[:, edges[i]:edges[i + 1]], w2_v[i][...])
            out = y_v[...] + gb * z
            if i + 1 < len(w2_v):
                y_v[...] = out
        with scope("s8_out"):
            o_ref[0] = out.astype(o_ref.dtype)

    def kernel(*refs):
        pl.run_scoped(functools.partial(body, *refs), sem=pltpu.SemaphoreType.DMA((S_W2 + len(w2_split),)))

    def fn(A_x, A_k_cache, A_v_cache, A_wq, A_wo, B_x, B_w1, B_b1, B_w2, c, w_mod):
        del B_x
        _, hkv, sk, dh = A_k_cache.shape
        assert A_x.shape[:2] == (1, 1) and (hkv, dh) == (HQ, DH)
        D = A_x.shape[-1]
        FF = B_w1.shape[1]
        W = min(4096, max(256, sk // 4))
        C = W // (2 * NC)
        kt = jnp.swapaxes(A_k_cache, 2, 3).reshape(hkv * dh, sk)
        vt = jnp.swapaxes(A_v_cache, 2, 3).reshape(hkv * dh, sk)
        b1 = B_b1.reshape(FF // 128, 128)
        return pl.pallas_call(
            kernel, name=name,
            out_shape=jax.ShapeDtypeStruct(A_x.shape, A_x.dtype),
            in_specs=[pl.BlockSpec(memory_space=pltpu.HBM)] * 10,
            out_specs=pl.BlockSpec(memory_space=pltpu.VMEM),
            scratch_shapes=[
                pltpu.VMEM(A_x.shape, BF16), pltpu.VMEM(c.shape, BF16), pltpu.VMEM(b1.shape, BF16),
                pltpu.VMEM(w_mod.shape, BF16), pltpu.VMEM(A_wq.shape, BF16),
                pltpu.VMEM((wo_a, D), BF16), pltpu.VMEM((A_wo.shape[0] - wo_a, D), BF16),
                pltpu.VMEM(B_w1.shape, BF16),
                pltpu.VMEM((2, 2, GR, C), BF16),
                pltpu.VMEM((NG, G, GR), F32), pltpu.VMEM((NC, 2, G, C), F32), pltpu.VMEM((NC, 2, G, C), F32),
                pltpu.VMEM((NG, 1, GR), F32), pltpu.VMEM((1, D), F32),
            ] + [pltpu.VMEM((r, D), BF16) for r in w2_split],
            compiler_params=pltpu.CompilerParams(vmem_limit_bytes=64 * 1024 * 1024),
        )(A_x, kt, vt, A_wq, A_wo, B_w1, b1, B_w2, c, w_mod)

    return fn


@jax.jit
def pallas_adaLN_cond__sliding_block_cached__dense_activation_mish__decode_kernel(
    A_x, A_k_cache, A_v_cache, A_wq, A_wo, B_x, B_w1, B_b1, B_w2, c, w_mod):
    return _make(w2_split=(896,512,128), vpu_tail=1)(A_x, A_k_cache, A_v_cache, A_wq, A_wo, B_x, B_w1, B_b1, B_w2, c, w_mod)
```

```python
import functools

import jax
import jax.numpy as jnp
from jax.experimental import pallas as pl
from jax.experimental.pallas import tpu as pltpu

F32 = jnp.float32
BF16 = jnp.bfloat16

HQ, DH = 32, 192
G = 8
GR = G * DH
NG = HQ // G
NC = 4
KV_ROWS = 32
WO_FIRST = 4608
W2_PARTS = (896, 512, 128)
W2_ROWS = 16
EPS = 1e-5

S_SMALL, S_WM, S_WQ, S_WOA, S_WOB, S_W1, S_W2 = range(2, 9)


def _layernorm(x):
    m = jnp.mean(x, axis=-1, keepdims=True)
    d = x - m
    v = jnp.mean(d * d, axis=-1, keepdims=True)
    return d / jnp.sqrt(v + EPS)


def _dot(a, b):
    return jnp.dot(a, b, preferred_element_type=F32)


def _dot_nt(a, b):
    return jax.lax.dot_general(a, b, (((1,), (1,)), ((), ())), preferred_element_type=F32)


def _loop(n, body):
    def step(i, carry):
        body(i)
        return carry
    jax.lax.fori_loop(0, n, step, 0)


def _body(x_hbm, kt_hbm, vt_hbm, wq_hbm, wo_hbm, w1_hbm, b1_hbm, w2_hbm, c_hbm, wm_hbm,
          o_ref,
          x_v, c_v, b1_v, wm_v, wq_v, woa_v, wob_v, w1_v, w2a_v, w2b_v, w2c_v,
          kv_v, q_v, s_v, a_v, y_v, coef_v, *, sem):
    D = x_v.shape[-1]
    FF = w1_v.shape[1]
    SK = kt_hbm.shape[1]
    C = kv_v.shape[3]
    W = 2 * NC * C

    def fetch(src, row0, dst, s, rows, cols, ways):
        n = dst.shape[0] // (rows * ways)
        nc = dst.shape[1] // cols
        assert (n * rows * ways, nc * cols) == dst.shape and ways % 2 == 0

        def sweep(i):
            for j in range(nc):
                for w in range(ways):
                    r = pl.multiple_of((w * n + i) * rows, rows)
                    pltpu.make_async_copy(src.at[pl.ds(row0 + r, rows), pl.ds(j * cols, cols)],
                                          dst.at[pl.ds(r, rows), pl.ds(j * cols, cols)],
                                          sem.at[s]).start(priority=w % 2)
        _loop(n, sweep)

    def fetch_kv(src, g, c):
        rows = pl.ds(pl.multiple_of(g * GR, GR), GR)
        strips = [src.at[rows, pl.ds(pl.multiple_of(SK - W + half * (W // 2) + c * C, C), C)]
                  for half in range(2)]

        def step(i):
            r = pl.ds(pl.multiple_of(i * KV_ROWS, KV_ROWS), KV_ROWS)
            for half in range(2):
                pltpu.make_async_copy(strips[half].at[r], kv_v.at[c % 2, half, r],
                                      sem.at[c % 2]).start(priority=half)
        _loop(GR // KV_ROWS, step)

    def landed(dst, s):
        pltpu.make_async_copy(dst, dst, sem.at[s]).wait()

    small = [pltpu.make_async_copy(src, dst, sem.at[S_SMALL])
             for src, dst in ((c_hbm, c_v), (x_hbm, x_v), (b1_hbm, b1_v))]
    fetch(wm_hbm, 0, wm_v, S_WM, 8, 1280, 10)
    for cp in small:
        cp.start()
    fetch(wq_hbm, 0, wq_v, S_WQ, 8, 2048, 20)

    for cp in small:
        cp.wait()
    landed(wm_v, S_WM)
    cv = c_v[...].astype(F32)
    mod = _dot((cv * jax.nn.sigmoid(cv)).astype(BF16), wm_v[...])
    sa, ca, ga, sb, cb, gb = (mod[:, i * D:(i + 1) * D] for i in range(6))
    x = x_v[0].astype(F32)
    h = (_layernorm(x) * (1.0 + ca) + sa).astype(BF16)

    fetch_kv(kt_hbm, 0, 0)
    landed(wq_v, S_WQ)
    row = jax.lax.broadcasted_iota(jnp.int32, (G, GR), 0)
    col = jax.lax.broadcasted_iota(jnp.int32, (G, GR), 1)
    own = (col >= row * DH) & (col < (row + 1) * DH)
    for g in range(NG):
        q = _dot(h, wq_v[:, g * GR:(g + 1) * GR])
        q_v[g] = jnp.where(own, jnp.broadcast_to(q, (G, GR)), 0.0)

    def group(g):
        qg = q_v[g].astype(BF16)

        def k_step(c):
            @pl.when(c + 1 < NC)
            def _():
                fetch_kv(kt_hbm, g, c + 1)

            @pl.when(c + 1 == NC)
            def _():
                fetch_kv(vt_hbm, g, 0)

            landed(kv_v.at[c % 2], c % 2)
            for half in range(2):
                s_v[c, half] = _dot(qg, kv_v[c % 2, half]) * DH ** -0.5

        _loop(NC, k_step)

        s = s_v[...]
        m = jnp.max(jnp.max(s, axis=(0, 1)), axis=-1, keepdims=True)
        e = jnp.exp(s - m[None, None])
        denom = jnp.sum(jnp.sum(e, axis=(0, 1)), axis=-1, keepdims=True)
        s_v[...] = e

        def v_step(c, acc):
            @pl.when(c + 1 < NC)
            def _():
                fetch_kv(vt_hbm, g, c + 1)

            @pl.when((c + 1 == NC) & (g + 1 < NG))
            def _():
                fetch_kv(kt_hbm, g + 1, 0)

            @pl.when((c + 1 == NC) & (g + 1 == NG))
            def _():
                fetch(wo_hbm, 0, woa_v, S_WOA, 16, D, 8)

            landed(kv_v.at[c % 2], c % 2)
            for half in range(2):
                acc = acc + _dot_nt(s_v[c, half].astype(BF16), kv_v[c % 2, half])
            return acc

        acc = jax.lax.fori_loop(0, NC, v_step, jnp.zeros((G, GR), F32))
        a_v[g] = jnp.sum(jnp.where(own, acc / denom, 0.0), axis=0, keepdims=True)

    _loop(NG, group)

    fetch(wo_hbm, WO_FIRST, wob_v, S_WOB, 16, D, 8)
    fetch(w1_hbm, 0, w1_v, S_W1, 8, FF, 4)
    a = jnp.concatenate([a_v[g] for g in range(NG)], axis=1).astype(BF16)
    landed(woa_v, S_WOA)
    y_v[...] = _dot(a[:, :WO_FIRST], woa_v[...])

    w2_v = (w2a_v, w2b_v, w2c_v)
    edge = [sum(W2_PARTS[:i]) for i in range(len(W2_PARTS) + 1)]
    for r0 in range(0, FF // 2, W2_ROWS):
        for queue in range(2):
            r = r0 + queue * (FF // 2)
            part = max(i for i in range(len(W2_PARTS)) if edge[i] <= r)
            pltpu.make_async_copy(w2_hbm.at[pl.ds(r, W2_ROWS)],
                                  w2_v[part].at[pl.ds(r - edge[part], W2_ROWS)],
                                  sem.at[S_W2 + part]).start(priority=queue)

    landed(wob_v, S_WOB)
    x1 = x + ga * (y_v[...] + _dot(a[:, WO_FIRST:], wob_v[...]))
    h2 = (_layernorm(x1) * (1.0 + cb) + sb).astype(BF16)
    y_v[...] = x1
    b1 = b1_v[...].astype(F32)
    b1 = jnp.concatenate([b1[j:j + 1, :] for j in range(FF // 128)], axis=1)
    landed(w1_v, S_W1)
    u = _dot(h2, w1_v[...]) + b1
    softplus = jnp.log1p(jnp.exp(-jnp.abs(u))) + jnp.where(u > 0, u, 0.0)
    act = (u * jnp.tanh(softplus)).astype(BF16)
    coef_v[...] = jnp.broadcast_to(act[:, edge[2]:].astype(F32), coef_v.shape).T

    for part in range(2):
        landed(w2_v[part], S_W2 + part)
        y_v[...] += gb * _dot(act[:, edge[part]:edge[part + 1]], w2_v[part][...])
    landed(w2c_v, S_W2 + 2)
    coef = coef_v[...]
    z = jnp.concatenate(
        [jnp.sum(w2c_v[:, j * 128:(j + 1) * 128].astype(F32) * coef, axis=0, keepdims=True)
         for j in range(D // 128)], axis=1)
    o_ref[0] = (y_v[...] + gb * z).astype(o_ref.dtype)


def _kernel(*refs):
    pl.run_scoped(functools.partial(_body, *refs),
                  sem=pltpu.SemaphoreType.DMA((S_W2 + len(W2_PARTS),)))


@jax.jit
def pallas_adaLN_cond__sliding_block_cached__dense_activation_mish__decode_kernel(
    A_x: jax.Array,
    A_k_cache: jax.Array,
    A_v_cache: jax.Array,
    A_wq: jax.Array,
    A_wo: jax.Array,
    B_x: jax.Array,
    B_w1: jax.Array,
    B_b1: jax.Array,
    B_w2: jax.Array,
    c: jax.Array,
    w_mod: jax.Array,
):
    del B_x
    _, hkv, sk, dh = A_k_cache.shape
    D = A_x.shape[-1]
    FF = B_w1.shape[1]
    W = min(4096, max(256, sk // 4))
    C = W // (2 * NC)
    assert A_x.shape[:2] == (1, 1) and (hkv, dh) == (HQ, DH)
    assert C % 128 == 0 and (sk - W) % C == 0 and sum(W2_PARTS) == FF and W2_PARTS[-1] == 128

    kt = jnp.swapaxes(A_k_cache, 2, 3).reshape(hkv * dh, sk)
    vt = jnp.swapaxes(A_v_cache, 2, 3).reshape(hkv * dh, sk)
    b1 = B_b1.reshape(FF // 128, 128)
    return pl.pallas_call(
        _kernel,
        name="adaln_attn_mish",
        out_shape=jax.ShapeDtypeStruct(A_x.shape, A_x.dtype),
        in_specs=[pl.BlockSpec(memory_space=pltpu.HBM)] * 10,
        out_specs=pl.BlockSpec(memory_space=pltpu.VMEM),
        scratch_shapes=[
            pltpu.VMEM(A_x.shape, BF16),
            pltpu.VMEM(c.shape, BF16),
            pltpu.VMEM(b1.shape, BF16),
            pltpu.VMEM(w_mod.shape, BF16),
            pltpu.VMEM(A_wq.shape, BF16),
            pltpu.VMEM((WO_FIRST, D), BF16),
            pltpu.VMEM((A_wo.shape[0] - WO_FIRST, D), BF16),
            pltpu.VMEM(B_w1.shape, BF16),
            *[pltpu.VMEM((r, D), BF16) for r in W2_PARTS],
            pltpu.VMEM((2, 2, GR, C), BF16),
            pltpu.VMEM((NG, G, GR), F32),
            pltpu.VMEM((NC, 2, G, C), F32),
            pltpu.VMEM((NG, 1, GR), F32),
            pltpu.VMEM((1, D), F32),
            pltpu.VMEM((128, 128), F32),
        ],
        compiler_params=pltpu.CompilerParams(vmem_limit_bytes=64 * 1024 * 1024),
    )(A_x, kt, vt, A_wq, A_wo, B_w1, b1, B_w2, c, w_mod)
```
